```python
import os as _os
_os.environ.setdefault("JAX_PLATFORMS", "cpu")
import jax
import jax.numpy as jnp

def _softmax(x, axis=-1):
    return jax.nn.softmax(x, axis=axis)
def _gelu(x):
    return jax.nn.gelu(x, approximate=True)
def _silu(x):
    return jax.nn.silu(x)
def _sigmoid(x):
    return jax.nn.sigmoid(x)
def _layernorm(x, axis=-1, eps=1e-5):
    m = jnp.mean(x, axis=axis, keepdims=True)
    v = jnp.var(x, axis=axis, keepdims=True)
    return (x - m) / jnp.sqrt(v + eps)
def _scatter_add(tgt, idx, src, axis=0):
    return tgt.at[idx].add(src)
def _segment_sum(src, seg, n):
    return jax.ops.segment_sum(src, seg, n)
class _Rng:
    def __init__(self, key):
        self._k = key
    def _next(self):
        self._k, sub = jax.random.split(self._k)
        return sub
    def normal(self, shape):
        return jax.random.normal(self._next(), shape, dtype=jnp.bfloat16)
    def randint(self, lo, hi, shape):
        return jax.random.randint(self._next(), shape, lo, hi, dtype=jnp.int32)
    def uniform(self, shape, lo=0.0, hi=1.0):
        return jax.random.uniform(self._next(), shape, jnp.bfloat16, lo, hi)
    def permutation(self, n):
        return jax.random.permutation(self._next(), n)


kernel_name = 'recurrent_scan__ssm_conv_s5__mixer_s_mlp__prompt'

def setup_inputs():
    _rng = _Rng(jax.random.key(int.from_bytes(__import__("os").urandom(4), "little")))
    _w = (lambda a: (lambda t: t.astype(jnp.bfloat16) if jnp.issubdtype(t.dtype, jnp.floating) else t)(jnp.asarray(a)))
    def _A_setup():
        B, S, D = 1, 2048, 640
        P = D
        Lambda_re = -0.5 * jnp.exp((lambda *s: _rng.normal(s) * 0.8)(P))
        Lambda_im = (lambda *s: _rng.normal(s) * 0.8)(P) * 1.0
        B_re = (lambda *s: _rng.normal(s) * 0.8)(P, D) * (D ** -0.5)
        B_im = (lambda *s: _rng.normal(s) * 0.8)(P, D) * (D ** -0.5)
        C_re = (lambda *s: _rng.normal(s) * 0.8)(D, P) * (P ** -0.5)
        C_im = (lambda *s: _rng.normal(s) * 0.8)(D, P) * (P ** -0.5)
        log_dt = (lambda *s: _rng.normal(s) * 0.8)(P) * 0.3 - 2.0
        Dskip = (lambda *s: _rng.normal(s) * 0.8)(D)
        return {
            "x": _w((lambda *s: _rng.normal(s) * 0.05)(B, S, D)),
            "Lambda_re": _w(Lambda_re),
            "Lambda_im": _w(Lambda_im),
            "B_re": _w(B_re),
            "B_im": _w(B_im),
            "C_re": _w(C_re),
            "C_im": _w(C_im),
            "log_dt": _w(log_dt),
            "Dskip": _w(Dskip),
        }
    _A_in = _A_setup()

    def _B_setup():
        B, S, D, F = 1, 2048, 640, 1536
        return {
            "x":  _w((lambda *s: _rng.normal(s) * 0.05)(B, S, D)),
            "w1": _w((lambda *s: _rng.normal(s) * 0.8)(D, D) * (D ** -0.5)),
            "w2": _w((lambda *s: _rng.normal(s) * 0.8)(D, D) * (D ** -0.5)),
            "w3": _w((lambda *s: _rng.normal(s) * 0.8)(D, F) * (D ** -0.5)),
            "w4": _w((lambda *s: _rng.normal(s) * 0.8)(F, D) * (F ** -0.5)),
        }
    _B_in = _B_setup()

    return {
        "A_x": _A_in["x"],
        "A_Lambda_re": _A_in["Lambda_re"],
        "A_Lambda_im": _A_in["Lambda_im"],
        "A_B_re": _A_in["B_re"],
        "A_B_im": _A_in["B_im"],
        "A_C_re": _A_in["C_re"],
        "A_C_im": _A_in["C_im"],
        "A_log_dt": _A_in["log_dt"],
        "A_Dskip": _A_in["Dskip"],
        "B_x": _B_in["x"],
        "B_w1": _B_in["w1"],
        "B_w2": _B_in["w2"],
        "B_w3": _B_in["w3"],
        "B_w4": _B_in["w4"],
    }

def reference(A_x, A_Lambda_re, A_Lambda_im, A_B_re, A_B_im, A_C_re, A_C_im, A_log_dt, A_Dskip, B_x, B_w1, B_w2, B_w3, B_w4):
    def _A_ref(x, Lambda_re, Lambda_im, B_re, B_im, C_re, C_im, log_dt, Dskip):
        Bsz, L, H = x.shape
        Lam = Lambda_re + 1j * Lambda_im
        Bmat = B_re + 1j * B_im
        Cmat = C_re + 1j * C_im
        dt = jnp.exp(log_dt)
        Lam_bar = jnp.exp(dt * Lam)
        B_bar = ((Lam_bar - 1.0) / Lam)[:, None] * Bmat
        Bu = jnp.einsum("bld,pd->blp", x + 0j, B_bar)
        h = jnp.zeros_like(Bu[:, 0, :])
        hs = []
        for t in range(L):
            h = Lam_bar[None, :] * h + Bu[:, t, :]
            hs.append(h)
        hseq = jnp.stack(hs, 1)
        y = 2.0 * jnp.einsum("blp,dp->bld", hseq, Cmat).real + x * Dskip[None, None, :]
        return y

    def _B_ref(x, w1, w2, w3, w4):
        B, S, D = x.shape
        h = _gelu(_layernorm(x, axis=-1) @ w1)
        c = D // 4
        g0 = jnp.pad(h[:, :, 0*c:1*c], ((0, 0), (1, 0), (0, 0)))[:, :S, :]
        g1 = jnp.pad(h[:, :, 1*c:2*c], ((0, 0), (0, 1), (0, 0)))[:, 1:, :]
        g2 = jnp.pad(h[:, :, 2*c:3*c], ((0, 0), (2, 0), (0, 0)))[:, :S, :]
        g3 = jnp.pad(h[:, :, 3*c:   ], ((0, 0), (0, 2), (0, 0)))[:, 2:, :]
        hs = jnp.concatenate([g0, g1, g2, g3], axis=-1) @ w2
        x1 = x + hs
        h2 = _gelu(_layernorm(x1, axis=-1) @ w3) @ w4
        return x1 + h2

    x = A_x
    xn = _layernorm(x, axis=-1)
    s = _A_ref(xn, A_Lambda_re, A_Lambda_im, A_B_re, A_B_im, A_C_re, A_C_im, A_log_dt, A_Dskip)
    g = _silu(_B_ref(xn, B_w1, B_w2, B_w3, B_w4))
    return x + s * g
```

```python
import math

import jax
import jax.numpy as jnp
from jax import lax
from jax.experimental import pallas as pl
from jax.experimental.pallas import tpu as pltpu

S, D, P, F = 2048, 640, 640, 1536
T = 256
LNG1 = 32
LNG2 = 32
SCOPES = 0
XN2SSA = 1
ORD = 0
L = 2
NB = L + 1
PRIO = 0
PFIRST = 1
PPRIO = 0
NBU = 2
N = S // T
NT = P // 128
EPS = 1e-5
C1 = math.sqrt(2.0 / math.pi)
C2 = C1 * 0.044715

f32 = jnp.float32
bf16 = jnp.bfloat16


def _gelu(x):
    hx = 0.5 * x
    t = jnp.tanh(x * (C1 + C2 * (x * x)))
    return hx + hx * t


def _silu(x):
    hx = 0.5 * x
    return hx + hx * jnp.tanh(hx)


_NT = (((1,), (1,)), ((), ()))


def dW1(a, b):
    return jnp.dot(a, b, preferred_element_type=f32)


def dW2(a, b):
    return jnp.dot(a, b, preferred_element_type=f32)


def dW3(a, b):
    return jnp.dot(a, b, preferred_element_type=f32)


def dW4(a, b):
    return jnp.dot(a, b, preferred_element_type=f32)


def dB(a, b):
    return lax.dot_general(a, b, _NT, preferred_element_type=f32)


def dC(a, b):
    return lax.dot_general(a, b, _NT, preferred_element_type=f32)


class _noscope:
    def __init__(self, n): pass
    def __enter__(self): pass
    def __exit__(self, *a): pass


scope = jax.named_scope if SCOPES else _noscope


def kernel(x_hbm, lre_hbm, lim_hbm, ldt_hbm, dsk_hbm,
           bre_hbm, bim_hbm, cre_hbm, cim_hbm, w1_hbm, w2_hbm, w3_hbm, w4_hbm,
           out_hbm,
           x_v, p0_v, p1_v, p2_v, p3_v, bre_v, bim_v, cre_v, cim_v, w1_v, w2_v, w3_v, w4_v, out_v,
           kc_ref, xn_ref, bu_all, hs_ref, g_ref, h1_ref, xn2_ref, zero_ref,
           xsem, wsem, osem, bar_sem):
    def cp(src, dst, sem):
        return pltpu.make_async_copy(src, dst, sem)

    def rows(i):
        return pl.ds(i * T, T)

    xcp = [cp(x_hbm.at[rows(i), :], x_v.at[rows(i), :], xsem.at[i]) for i in range(N)]
    p_v = (p0_v, p1_v, p2_v, p3_v)
    pcp = [cp(h, p_v[n], wsem.at[n]) for n, h in enumerate((lre_hbm, lim_hbm, ldt_hbm, dsk_hbm))]
    w1cp = cp(w1_hbm, w1_v, wsem.at[4])
    bcp = [cp(bre_hbm, bre_v, wsem.at[5]), cp(bim_hbm, bim_v, wsem.at[10])]
    ccp = [cp(cre_hbm, cre_v, wsem.at[6]), cp(cim_hbm, cim_v, wsem.at[11])]
    w2cp = cp(w2_hbm, w2_v, wsem.at[7])
    w3cp = cp(w3_hbm, w3_v, wsem.at[8])
    w4cp = cp(w4_hbm, w4_v, wsem.at[9])
    ocp = [cp(out_v.at[rows(i), :], out_hbm.at[rows(i), :], osem.at[i]) for i in range(N)]

    def ln_chain(load, store, n, lng):
        never = jnp.broadcast_to(zero_ref[0:1, 0:1] != 0.0, (lng, 1))
        prev = None
        for g in range(n // lng):
            xg = load(lng * g, lng)
            m = jnp.sum(xg, axis=-1, keepdims=True) * (1.0 / D)
            if prev is not None:
                m = jnp.where(never, prev, m)
            d = xg - m
            v = jnp.sum(d * d, axis=-1, keepdims=True) * (1.0 / D)
            r = lax.rsqrt(v + EPS)
            prev = r
            store(lng * g, lng, (d * r).astype(bf16))

    def ln1(i, lng):
        def load(o, n):
            return x_v[pl.ds(i * T + o, n), :].astype(f32)

        def store(o, n, val):
            xn_ref[pl.ds(i * T + o, n), :] = val
        ln_chain(load, store, T, lng)

    def mm_w1(i):
        h1_ref[pl.ds(8 + i * T, T), :] = _gelu(dW1(xn_ref[rows(i), :], w1_v[...]))

    def mm_b(i, part):
        bu_ref = bu_all.at[i % NB]
        bu_ref[:, part * P:(part + 1) * P] = dB(xn_ref[rows(i), :], (bre_v, bim_v)[part][...])

    def prep_scan():
        ld = lambda n: jnp.broadcast_to(p_v[n][...].astype(f32).reshape(1, P), (8, P))
        lre, lim = ld(0), ld(1)
        dt = jnp.exp(ld(2))
        kc_ref[10] = ld(3)
        zr = dt * lre
        zi = dt * lim
        row = lax.broadcasted_iota(jnp.int32, (8, P), 0)
        k = (row + 1).astype(f32)
        mag = jnp.exp(k * zr)
        pr = mag * jnp.cos(k * zi)
        pi = mag * jnp.sin(k * zi)
        kc_ref[6] = jnp.where(row == 0, jnp.broadcast_to(pr[0:1], (8, P)), 0.0)
        kc_ref[7] = jnp.where(row == 0, jnp.broadcast_to(pi[0:1], (8, P)), 0.0)
        for n, d in enumerate((1, 2, 4)):
            kc_ref[2 * n] = jnp.where(row >= d, jnp.broadcast_to(pr[d - 1:d], (8, P)), 0.0)
            kc_ref[2 * n + 1] = jnp.where(row >= d, jnp.broadcast_to(pi[d - 1:d], (8, P)), 0.0)
        ar = jnp.broadcast_to(pr[0:1], (8, P)) - 1.0
        ai = jnp.broadcast_to(pi[0:1], (8, P))
        den = 2.0 / (lre * lre + lim * lim)
        kc_ref[8] = (ar * lre + ai * lim) * den
        kc_ref[9] = (ai * lre - ar * lim) * den
        kc_ref[11] = jnp.zeros((8, P), f32)
        kc_ref[12] = jnp.zeros((8, P), f32)

    def scan(i):
        bu_ref = bu_all.at[i % NB]
        never = zero_ref[...] != 0.0
        last = None
        for j in range(NT):
            sl = slice(128 * j, 128 * (j + 1))
            k = [kc_ref[n, :, sl] for n in range(10)]
            cr = kc_ref[11, :, sl]
            ci = kc_ref[12, :, sl]
            if last is not None:
                cr = jnp.where(never, last, cr)
            for r2 in range(T // 16):
                hh = []
                for r in (2 * r2, 2 * r2 + 1):
                    ur = bu_ref[8 * r:8 * r + 8, sl]
                    ui = bu_ref[8 * r:8 * r + 8, P + 128 * j:P + 128 * (j + 1)]
                    rr = pltpu.roll(cr, 1, 0)
                    ri = pltpu.roll(ci, 1, 0)
                    hr = (k[8] * ur - k[9] * ui) + (k[6] * rr + k[7] * ri)
                    hi = (k[6] * ri - k[7] * rr) - (k[8] * ui + k[9] * ur)
                    for n, d in enumerate((1, 2, 4)):
                        rr = pltpu.roll(hr, d, 0)
                        ri = pltpu.roll(hi, d, 0)
                        hr, hi = (hr + (k[2 * n] * rr + k[2 * n + 1] * ri),
                                  hi + (k[2 * n] * ri - k[2 * n + 1] * rr))
                    cr, ci = hr, hi
                    hh.append((hr, hi))
                rs = slice(16 * r2, 16 * r2 + 16)
                hs_ref[rs, sl] = jnp.concatenate([hh[0][0], hh[1][0]], 0).astype(bf16)
                hs_ref[rs, P + 128 * j:P + 128 * (j + 1)] = jnp.concatenate([hh[0][1], hh[1][1]], 0).astype(bf16)
            kc_ref[11, :, sl] = cr
            kc_ref[12, :, sl] = ci
            last = cr

    def mm_w2(i):
        lane = lax.broadcasted_iota(jnp.int32, (T, 128), 1)

        def sh(j, s):
            return h1_ref[pl.ds(8 + i * T - s, T), 128 * j:128 * (j + 1)]

        g = jnp.concatenate([
            sh(0, 1),
            jnp.where(lane < 32, sh(1, 1), sh(1, -1)),
            jnp.where(lane < 64, sh(2, -1), sh(2, 2)),
            jnp.where(lane < 96, sh(3, 2), sh(3, -2)),
            sh(4, -2)], axis=1).astype(bf16)
        return xn_ref[rows(i), :].astype(f32) + dW2(g, w2_v[...])

    def ln2(x1, lng):
        outs = []

        def store(o, n, val):
            if XN2SSA:
                outs.append(val)
            else:
                xn2_ref[pl.ds(o, n), :] = val
        ln_chain(lambda o, n: x1[o:o + n], store, T, lng)
        return jnp.concatenate(outs, 0) if XN2SSA else None

    def mm_w3(xn2):
        if xn2 is None:
            xn2 = xn2_ref[...]
        return _gelu(dW3(xn2, w3_v[...])).astype(bf16)

    def mm_w4(x1, h3):
        g_ref[...] = _silu(x1 + dW4(h3, w4_v[...]))

    def mm_c(i):
        gg = g_ref[...]
        s = dC(hs_ref[:, 0:P], cre_v[...]) + dC(hs_ref[:, P:2 * P], cim_v[...]) + xn_ref[rows(i), :].astype(f32) * kc_ref[10, 0:1, :]
        out_v[rows(i), :] = x_v[rows(i), :].astype(f32) + s * gg

    def fence():
        pl.semaphore_signal(bar_sem, 1)
        pl.semaphore_wait(bar_sem, 1)

    with scope("starts"):
        order = [xcp[0], w1cp] + xcp[1:L + 1] + bcp[:1] + pcp + bcp[1:] + [w2cp, w3cp, w4cp] + ccp + xcp[L + 1:]
        for c in order:
            c.start()
            fence()
        h1_ref[0:8, :] = jnp.zeros((8, D), f32)
        h1_ref[8 + S:16 + S, :] = jnp.zeros((8, D), f32)
        zero_ref[...] = jnp.zeros((8, 128), f32)
    with scope("pro_x0"):
        xcp[0].wait()
        ln1(0, T)
    with scope("pro_w1"):
        w1cp.wait()
        mm_w1(0)
    for i in range(1, L):
        with scope(f"pro_w1_{i}"):
            xcp[i].wait()
            ln1(i, T)
            mm_w1(i)
    with scope("pro_b"):
        xcp[L].wait()
        bcp[0].wait()
        ln1(L, LNG1)
        for i in range(L):
            mm_b(i, 0)
        for c in pcp:
            c.wait()
        bcp[1].wait()
        for i in range(L):
            mm_b(i, 1)
        prep_scan()
    waited = set()
    for i in range(N):
        with scope(f"it{i}"):
            if i >= 1 and i + L + 1 < N:
                xcp[i + L + 1].wait()
            elif i >= 3:
                ocp[i - 3].wait()
                waited.add(i - 3)
            elif i >= 1:
                fence()
            if i >= 2:
                ocp[i - 2].start()
            if i + L < N:
                mm_w1(i + L)
            if i >= 1 and i + L < N:
                mm_b(i + L, 0)
                mm_b(i + L, 1)
            if i == 0:
                w2cp.wait()
            x1 = mm_w2(i)
            if i == 0:
                w3cp.wait()
                mm_b(L, 0)
                mm_b(L, 1)
            xn2 = ln2(x1, LNG2)
            if i >= 1:
                mm_c(i - 1)
            if i >= 1 and i + L + 1 < N:
                ln1(i + L + 1, LNG1)
            h3 = mm_w3(xn2)
            if i == 0:
                w4cp.wait()
                if L + 1 < N:
                    xcp[L + 1].wait()
                    ln1(L + 1, LNG1)
            mm_w4(x1, h3)
            scan(i)
        if i == 0:
            with scope("cwait"):
                for c in ccp:
                    c.wait()
    with scope("epi"):
        fence()
        ocp[N - 2].start()
        mm_c(N - 1)
        ocp[N - 1].start()
        for i, c in enumerate(ocp):
            if i not in waited:
                c.wait()


@jax.jit
def pallas_recurrent_scan__ssm_conv_s5__mixer_s_mlp__prompt_kernel(
    A_x, A_Lambda_re, A_Lambda_im, A_B_re, A_B_im, A_C_re, A_C_im, A_log_dt, A_Dskip,
    B_x, B_w1, B_w2, B_w3, B_w4,
):
    x = A_x.reshape(S, D)
    ins = (x, A_Lambda_re, A_Lambda_im, A_log_dt, A_Dskip, A_B_re, A_B_im, A_C_re, A_C_im, B_w1, B_w2, B_w3, B_w4)
    anyspec = pl.BlockSpec(memory_space=pl.ANY)
    out = pl.pallas_call(
        kernel,
        in_specs=[anyspec] * len(ins),
        out_specs=anyspec,
        out_shape=jax.ShapeDtypeStruct((S, D), f32),
        scratch_shapes=[
            pltpu.VMEM((S, D), bf16),
            pltpu.VMEM((P,), bf16),
            pltpu.VMEM((P,), bf16),
            pltpu.VMEM((P,), bf16),
            pltpu.VMEM((P,), bf16),
            pltpu.VMEM((P, D), bf16),
            pltpu.VMEM((P, D), bf16),
            pltpu.VMEM((D, P), bf16),
            pltpu.VMEM((D, P), bf16),
            pltpu.VMEM((D, D), bf16),
            pltpu.VMEM((D, D), bf16),
            pltpu.VMEM((D, F), bf16),
            pltpu.VMEM((F, D), bf16),
            pltpu.VMEM((S, D), f32),
            pltpu.VMEM((13, 8, P), f32),
            pltpu.VMEM((S, D), bf16),
            pltpu.VMEM((NB, T, 2 * P), f32),
            pltpu.VMEM((T, 2 * P), bf16),
            pltpu.VMEM((T, D), f32),
            pltpu.VMEM((S + 16, D), f32),
            pltpu.VMEM((T, D), bf16),
            pltpu.VMEM((8, 128), f32),
            pltpu.SemaphoreType.DMA((N,)),
            pltpu.SemaphoreType.DMA((12,)),
            pltpu.SemaphoreType.DMA((N,)),
            pltpu.SemaphoreType.REGULAR,
        ],
        compiler_params=pltpu.CompilerParams(
            vmem_limit_bytes=100 * 1024 * 1024,
        ),
    )(*ins)
    return out.reshape(1, S, D)
```

```python
import math

import jax
import jax.numpy as jnp
from jax import lax
from jax.experimental import pallas as pl
from jax.experimental.pallas import tpu as pltpu

S, D, P, F = 2048, 640, 640, 1536
T = 256
N = S // T
L = 3
NB = L + 1
NT = P // 128
LNG = 32
WS = 256
OSPLIT = 512
EPS = 1e-5
C1 = math.sqrt(2.0 / math.pi)
C2 = C1 * 0.044715

f32 = jnp.float32
bf16 = jnp.bfloat16


def _gelu(x):
    hx = 0.5 * x
    t = jnp.tanh(x * (C1 + C2 * (x * x)))
    return hx + hx * t


def _silu(x):
    hx = 0.5 * x
    return hx + hx * jnp.tanh(hx)


def _nn(a, b):
    return jnp.dot(a, b, preferred_element_type=f32)


def _nt(a, b):
    return lax.dot_general(a, b, (((1,), (1,)), ((), ())), preferred_element_type=f32)


def kernel(x_hbm, lre_hbm, lim_hbm, ldt_hbm, dsk_hbm,
           bre_hbm, bim_hbm, cre_hbm, cim_hbm, w1_hbm, w2_hbm, w3_hbm, w4_hbm,
           out_hbm,
           x_v, p0_v, p1_v, p2_v, p3_v, bre_v, bim_v, cre_v, cim_v, w1_v, w2_v, w3_v, w4_v, out_v,
           kc_ref, xn_ref, bu_all, hs_ref, g_ref, x1_ref, h1_ref, xn2_ref, zero_ref,
           xsem, wsem, osem, bar_sem):
    def cp(src, dst, sem):
        return pltpu.make_async_copy(src, dst, sem)

    def rows(i):
        return pl.ds(i * T, T)

    xcp = [cp(x_hbm.at[rows(i), :], x_v.at[rows(i), :], xsem.at[i]) for i in range(N)]
    p_v = (p0_v, p1_v, p2_v, p3_v)
    pcp = [cp(h, p_v[n], wsem.at[n]) for n, h in enumerate((lre_hbm, lim_hbm, ldt_hbm, dsk_hbm))]
    w1cp = [cp(w1_hbm.at[:, pl.ds(0, WS)], w1_v.at[:, pl.ds(0, WS)], wsem.at[4]),
            cp(w1_hbm.at[:, pl.ds(WS, D - WS)], w1_v.at[:, pl.ds(WS, D - WS)], wsem.at[12])]
    bcp = [cp(bre_hbm, bre_v, wsem.at[5]), cp(bim_hbm, bim_v, wsem.at[10])]
    ccp = [cp(cre_hbm, cre_v, wsem.at[6]), cp(cim_hbm, cim_v, wsem.at[11])]
    w2cp = cp(w2_hbm, w2_v, wsem.at[7])
    w3cp = cp(w3_hbm, w3_v, wsem.at[8])
    w4cp = cp(w4_hbm, w4_v, wsem.at[9])
    ocp = [cp(out_v.at[rows(i), :], out_hbm.at[rows(i), :], osem.at[i]) for i in range(N - 1)]

    def ln_chain(load, store, n, lng, prev=None):
        never = jnp.broadcast_to(zero_ref[0:1, 0:1] != 0.0, (lng, 1))
        for g in range(n // lng):
            xg = load(lng * g, lng)
            m = jnp.sum(xg, axis=-1, keepdims=True) * (1.0 / D)
            if prev is not None:
                m = jnp.where(never, prev, m)
            d = xg - m
            v = jnp.sum(d * d, axis=-1, keepdims=True) * (1.0 / D)
            r = lax.rsqrt(v + EPS)
            prev = r
            store(lng * g, lng, (d * r).astype(bf16))
        return prev

    def ln1(i, lng, prev=None):
        def load(o, n):
            return x_v[pl.ds(i * T + o, n), :].astype(f32)

        def store(o, n, val):
            xn_ref[pl.ds(i * T + o, n), :] = val
        ln_chain(load, store, T, lng, prev)

    def mm_w1(i, c0=0, c1=D):
        h1_ref[pl.ds(8 + i * T, T), c0:c1] = _gelu(_nn(xn_ref[rows(i), :], w1_v[:, c0:c1]))

    def mm_b(i, part):
        bu_ref = bu_all.at[i % NB]
        bu_ref[:, part * P:(part + 1) * P] = _nt(xn_ref[rows(i), :], (bre_v, bim_v)[part][...])

    def prep_scan():
        ld = lambda n: jnp.broadcast_to(p_v[n][...].astype(f32).reshape(1, P), (8, P))
        lre, lim = ld(0), ld(1)
        dt = jnp.exp(ld(2))
        kc_ref[10] = ld(3)
        zr = dt * lre
        zi = dt * lim
        row = lax.broadcasted_iota(jnp.int32, (8, P), 0)
        k = (row + 1).astype(f32)
        mag = jnp.exp(k * zr)
        pr = mag * jnp.cos(k * zi)
        pi = mag * jnp.sin(k * zi)
        kc_ref[6] = jnp.where(row == 0, jnp.broadcast_to(pr[0:1], (8, P)), 0.0)
        kc_ref[7] = jnp.where(row == 0, jnp.broadcast_to(pi[0:1], (8, P)), 0.0)
        for n, d in enumerate((1, 2, 4)):
            kc_ref[2 * n] = jnp.where(row >= d, jnp.broadcast_to(pr[d - 1:d], (8, P)), 0.0)
            kc_ref[2 * n + 1] = jnp.where(row >= d, jnp.broadcast_to(pi[d - 1:d], (8, P)), 0.0)
        ar = jnp.broadcast_to(pr[0:1], (8, P)) - 1.0
        ai = jnp.broadcast_to(pi[0:1], (8, P))
        den = 2.0 / (lre * lre + lim * lim)
        kc_ref[8] = (ar * lre + ai * lim) * den
        kc_ref[9] = (ai * lre - ar * lim) * den
        kc_ref[11] = jnp.zeros((8, P), f32)
        kc_ref[12] = jnp.zeros((8, P), f32)

    def scan(i):
        bu_ref = bu_all.at[i % NB]
        never = zero_ref[...] != 0.0
        last = None
        for j in range(NT):
            sl = slice(128 * j, 128 * (j + 1))
            k = [kc_ref[n, :, sl] for n in range(10)]
            cr = kc_ref[11, :, sl]
            ci = kc_ref[12, :, sl]
            if last is not None:
                cr = jnp.where(never, last, cr)
            for r2 in range(T // 16):
                hh = []
                for r in (2 * r2, 2 * r2 + 1):
                    ur = bu_ref[8 * r:8 * r + 8, sl]
                    ui = bu_ref[8 * r:8 * r + 8, P + 128 * j:P + 128 * (j + 1)]
                    rr = pltpu.roll(cr, 1, 0)
                    ri = pltpu.roll(ci, 1, 0)
                    hr = (k[8] * ur - k[9] * ui) + (k[6] * rr + k[7] * ri)
                    hi = (k[6] * ri - k[7] * rr) - (k[8] * ui + k[9] * ur)
                    for n, d in enumerate((1, 2, 4)):
                        rr = pltpu.roll(hr, d, 0)
                        ri = pltpu.roll(hi, d, 0)
                        hr, hi = (hr + (k[2 * n] * rr + k[2 * n + 1] * ri),
                                  hi + (k[2 * n] * ri - k[2 * n + 1] * rr))
                    cr, ci = hr, hi
                    hh.append((hr, hi))
                rs = slice(16 * r2, 16 * r2 + 16)
                hs_ref[i % 2, rs, sl] = jnp.concatenate([hh[0][0], hh[1][0]], 0).astype(bf16)
                hs_ref[i % 2, rs, P + 128 * j:P + 128 * (j + 1)] = jnp.concatenate([hh[0][1], hh[1][1]], 0).astype(bf16)
            kc_ref[11, :, sl] = cr
            kc_ref[12, :, sl] = ci
            last = cr

    def mm_w2(i):
        lane = lax.broadcasted_iota(jnp.int32, (T, 128), 1)

        def sh(j, s):
            return h1_ref[pl.ds(8 + i * T - s, T), 128 * j:128 * (j + 1)]

        g = jnp.concatenate([
            sh(0, 1),
            jnp.where(lane < 32, sh(1, 1), sh(1, -1)),
            jnp.where(lane < 64, sh(2, -1), sh(2, 2)),
            jnp.where(lane < 96, sh(3, 2), sh(3, -2)),
            sh(4, -2)], axis=1).astype(bf16)
        return xn_ref[rows(i), :].astype(f32) + _nn(g, w2_v[...])

    def ln2(x1, ssa):
        outs = []

        def store(o, n, val):
            if ssa:
                outs.append(val)
            else:
                xn2_ref[pl.ds(o, n), :] = val
        last = ln_chain(lambda o, n: x1[o:o + n], store, T, LNG)
        return (jnp.concatenate(outs, 0) if ssa else None), last

    def mm_w3(xn2):
        if xn2 is None:
            xn2 = xn2_ref[...]
        return _gelu(_nn(xn2, w3_v[...])).astype(bf16)

    def mm_w4(x1, h3):
        g_ref[...] = _silu(x1 + _nn(h3, w4_v[...]))

    def mm_c(i, c0=0, c1=D):
        gg = g_ref[:, c0:c1]
        s = (_nt(hs_ref[i % 2, :, 0:P], cre_v[c0:c1, :]) + _nt(hs_ref[i % 2, :, P:2 * P], cim_v[c0:c1, :])
             + xn_ref[rows(i), c0:c1].astype(f32) * kc_ref[10, 0:1, c0:c1])
        out_v[rows(i), c0:c1] = x_v[rows(i), c0:c1].astype(f32) + s * gg

    def fence():
        pl.semaphore_signal(bar_sem, 1)
        pl.semaphore_wait(bar_sem, 1)

    tail = pl.ds((N - 1) * T, T)
    olast = [cp(out_v.at[tail, pl.ds(0, OSPLIT)], out_hbm.at[tail, pl.ds(0, OSPLIT)], osem.at[N - 1]),
             cp(out_v.at[tail, pl.ds(OSPLIT, D - OSPLIT)], out_hbm.at[tail, pl.ds(OSPLIT, D - OSPLIT)], wsem.at[13])]

    for c in (pcp + xcp[:2] + w1cp + [bcp[0], xcp[2], xcp[3], bcp[1], w2cp, w3cp, w4cp, xcp[4]]
              + ccp + xcp[5:]):
        c.start()
        fence()
    h1_ref[0:8, :] = jnp.zeros((8, D), f32)
    h1_ref[8 + S:16 + S, :] = jnp.zeros((8, D), f32)
    zero_ref[...] = jnp.zeros((8, 128), f32)

    for c in pcp:
        c.wait()
    prep_scan()
    xcp[0].wait()
    ln1(0, T)
    xcp[1].wait()
    ln1(1, T)
    w1cp[0].wait()
    mm_w1(0, 0, WS)
    mm_w1(1, 0, WS)
    w1cp[1].wait()
    mm_w1(0, WS, D)
    mm_w1(1, WS, D)
    bcp[0].wait()
    mm_b(0, 0)
    mm_b(1, 0)
    xcp[2].wait()
    xcp[3].wait()
    bcp[1].wait()
    ln1(2, LNG)
    ln1(3, LNG)
    mm_b(0, 1)
    mm_b(1, 1)
    mm_w1(2)
    mm_b(2, 0)
    mm_b(2, 1)
    w2cp.wait()
    mm_w1(3)
    x1 = mm_w2(0)
    mm_b(3, 0)
    mm_b(3, 1)
    x1_ref[...] = x1
    ln2(x1, ssa=False)
    w3cp.wait()
    w4cp.wait()
    xcp[4].wait()
    scan(0)
    ln1(4, LNG)
    mm_w4(x1_ref[...], mm_w3(None))

    started, waited = set(), set()

    def ostart(upto):
        pending = started - waited
        if pending:
            ocp[min(pending)].wait()
            waited.add(min(pending))
        else:
            fence()
        for n in range(upto + 1):
            if n not in started:
                ocp[n].start()
                started.add(n)

    for c in ccp + xcp[5:]:
        c.wait()
    for i in range(1, N):
        if i in (3, 5):
            ostart(i - 2)
        if i + L < N:
            mm_w1(i + L)
        if i < N - 1:
            scan(i)
        if i + L < N:
            mm_b(i + L, 0)
            mm_b(i + L, 1)
        x1 = mm_w2(i)
        if i == N - 1:
            x1_ref[...] = x1
        xn2, last = ln2(x1, ssa=i < N - 1)
        mm_c(i - 1)
        if i + L + 1 < N:
            ln1(i + L + 1, LNG, last)
        if i == N - 1:
            ostart(N - 2)
            scan(i)
            x1 = x1_ref[...]
        mm_w4(x1, mm_w3(xn2))

    mm_c(N - 1, 0, OSPLIT)
    fence()
    olast[0].start()
    mm_c(N - 1, OSPLIT, D)
    olast[1].start()
    for n, c in enumerate(ocp):
        if n not in waited:
            c.wait()
    for c in olast:
        c.wait()


@jax.jit
def pallas_recurrent_scan__ssm_conv_s5__mixer_s_mlp__prompt_kernel(
    A_x, A_Lambda_re, A_Lambda_im, A_B_re, A_B_im, A_C_re, A_C_im, A_log_dt, A_Dskip,
    B_x, B_w1, B_w2, B_w3, B_w4,
):
    x = A_x.reshape(S, D)
    ins = (x, A_Lambda_re, A_Lambda_im, A_log_dt, A_Dskip, A_B_re, A_B_im, A_C_re, A_C_im, B_w1, B_w2, B_w3, B_w4)
    anyspec = pl.BlockSpec(memory_space=pl.ANY)
    out = pl.pallas_call(
        kernel,
        in_specs=[anyspec] * len(ins),
        out_specs=anyspec,
        out_shape=jax.ShapeDtypeStruct((S, D), f32),
        scratch_shapes=[
            pltpu.VMEM((S, D), bf16),
            pltpu.VMEM((P,), bf16),
            pltpu.VMEM((P,), bf16),
            pltpu.VMEM((P,), bf16),
            pltpu.VMEM((P,), bf16),
            pltpu.VMEM((P, D), bf16),
            pltpu.VMEM((P, D), bf16),
            pltpu.VMEM((D, P), bf16),
            pltpu.VMEM((D, P), bf16),
            pltpu.VMEM((D, D), bf16),
            pltpu.VMEM((D, D), bf16),
            pltpu.VMEM((D, F), bf16),
            pltpu.VMEM((F, D), bf16),
            pltpu.VMEM((S, D), f32),
            pltpu.VMEM((13, 8, P), f32),
            pltpu.VMEM((S, D), bf16),
            pltpu.VMEM((NB, T, 2 * P), f32),
            pltpu.VMEM((2, T, 2 * P), bf16),
            pltpu.VMEM((T, D), f32),
            pltpu.VMEM((T, D), f32),
            pltpu.VMEM((S + 16, D), f32),
            pltpu.VMEM((T, D), bf16),
            pltpu.VMEM((8, 128), f32),
            pltpu.SemaphoreType.DMA((N,)),
            pltpu.SemaphoreType.DMA((14,)),
            pltpu.SemaphoreType.DMA((N,)),
            pltpu.SemaphoreType.REGULAR,
        ],
        compiler_params=pltpu.CompilerParams(
            vmem_limit_bytes=100 * 1024 * 1024,
        ),
    )(*ins)
    return out.reshape(1, S, D)
```
